```python
import os as _os
_os.environ.setdefault('JAX_PLATFORMS', 'cpu')
import jax
import jax.numpy as jnp

def _softmax(x, axis=-1):
    return jax.nn.softmax(x, axis=axis)

def _gelu(x):
    return jax.nn.gelu(x, approximate=True)

def _silu(x):
    return jax.nn.silu(x)

def _sigmoid(x):
    return jax.nn.sigmoid(x)

def _layernorm(x, axis=-1, eps=1e-05):
    m = jnp.mean(x, axis=axis, keepdims=True)
    v = jnp.var(x, axis=axis, keepdims=True)
    return (x - m) / jnp.sqrt(v + eps)

def _scatter_add(tgt, idx, src, axis=0):
    return tgt.at[idx].add(src)

def _segment_sum(src, seg, n):
    return jax.ops.segment_sum(src, seg, n)

class _Rng:

    def __init__(self, key):
        self._k = key

    def _next(self):
        self._k, sub = jax.random.split(self._k)
        return sub

    def normal(self, shape):
        return jax.random.normal(self._next(), shape, dtype=jnp.bfloat16)

    def randint(self, lo, hi, shape):
        return jax.random.randint(self._next(), shape, lo, hi, dtype=jnp.int32)

    def uniform(self, shape, lo=0.0, hi=1.0):
        return jax.random.uniform(self._next(), shape, jnp.bfloat16, lo, hi)

    def permutation(self, n):
        return jax.random.permutation(self._next(), n)
kernel_name = 'adaLN_cond__mha_block__geglu_ffn__prompt'

def setup_inputs():
    _rng = _Rng(jax.random.key(int.from_bytes(__import__("os").urandom(4), "little")))
    _w = lambda a: (lambda t: t.astype(jnp.bfloat16) if jnp.issubdtype(t.dtype, jnp.floating) else t)(jnp.asarray(a))

    def _A_setup():
        B, S, D, H = (1, 2048, 640, 32)
        return {'x': _w((lambda *s: _rng.normal(s) * 0.05)(B, S, D)), 'wqkv': _w((lambda *s: _rng.normal(s) * 0.05)(D, 3 * D)), 'wo': _w((lambda *s: _rng.normal(s) * 0.05)(D, D))}
    _A_in = _A_setup()

    def _B_setup():
        B, S, D, F = (1, 2048, 640, 1728)
        return {'x': _w((lambda *s: _rng.normal(s) * 0.05)(B, S, D)), 'w_gate': _w((lambda *s: _rng.normal(s) * 0.05)(D, F)), 'w_up': _w((lambda *s: _rng.normal(s) * 0.05)(D, F)), 'w_down': _w((lambda *s: _rng.normal(s) * 0.05)(F, D))}
    _B_in = _B_setup()
    return {'A_x': _A_in['x'], 'A_wqkv': _A_in['wqkv'], 'A_wo': _A_in['wo'], 'B_x': _B_in['x'], 'B_w_gate': _B_in['w_gate'], 'B_w_up': _B_in['w_up'], 'B_w_down': _B_in['w_down'], 'c': _w((lambda *s: _rng.normal(s) * 0.05)(1, 640) * 8.0), 'w_mod': _w((lambda *s: _rng.normal(s) * 0.05)(640, 6 * 640) * 640 ** (-0.5) * 8.0)}

def reference(A_x, A_wqkv, A_wo, B_x, B_w_gate, B_w_up, B_w_down, c, w_mod):

    def _A_ref(x, wqkv, wo):
        B, S, D = x.shape
        H = 32
        Dh = D // H
        qkv = (lambda x, *d: x.transpose(*d))((x @ wqkv).reshape(B, S, 3, H, Dh), 2, 0, 3, 1, 4)
        q, k, v = (qkv[0], qkv[1], qkv[2])
        scores = jnp.einsum('bhqd,bhkd->bhqk', q, k) * Dh ** (-0.5)
        p = _softmax(scores, axis=-1)
        o = jnp.einsum('bhqk,bhkd->bhqd', p, v)
        return (lambda x, *d: x.transpose(*d))(o, 0, 2, 1, 3).reshape(B, S, D) @ wo

    def _B_ref(x, w_gate, w_up, w_down):
        return _gelu(x @ w_gate) * (x @ w_up) @ w_down
    x = A_x
    mod = (_silu(c) @ w_mod).reshape(c.shape[0], 6, 1, -1)
    sa, ca, ga, sb, cb, gb = (mod[:, 0].copy(), mod[:, 1].copy(), mod[:, 2].copy(), mod[:, 3].copy(), mod[:, 4].copy(), mod[:, 5].copy())
    h = _layernorm(x, axis=-1) * (1 + ca) + sa
    x = x + ga * _A_ref(h, A_wqkv, A_wo)
    h = _layernorm(x, axis=-1) * (1 + cb) + sb
    x = x + gb * _B_ref(h, B_w_gate, B_w_up, B_w_down)
    return x
```

```python
import jax
import jax.numpy as jnp
import jax.experimental.pallas as pl
import jax.experimental.pallas.tpu as pltpu

S = 2048
D = 640
H = 32
DH = 20
F = 1728
FA = 1664
FT = F - FA
TQ = 512
NQ = S // TQ
KC = 128
SKEW = 2
UPB = 8
RC = 256
PB = 256
PRC = 128
FB = 256
FRC = 128
HPW = 6
NW = 6
EPS = 1e-5
LOG2E = 1.4426950408889634
QSCALE = (DH ** -0.5) * LOG2E

_NT = (((1,), (1,)), ((), ()))
_BF = jnp.bfloat16
_F32 = jnp.float32


class _scope:
    enabled = False

    def __init__(self, name):
        self._cm = jax.named_scope(name) if _scope.enabled else None

    def __enter__(self):
        if self._cm is not None:
            self._cm.__enter__()

    def __exit__(self, *a):
        if self._cm is not None:
            self._cm.__exit__(*a)


def _win_start(w):
    return min(w * HPW * DH, D - 128)


def _layernorm(x):
    m = jnp.mean(x, axis=-1, keepdims=True)
    xc = x - m
    v = jnp.mean(xc * xc, axis=-1, keepdims=True)
    return xc * jax.lax.rsqrt(v + EPS)


def _kernel(x_hbm, wqkv_hbm, wo_hbm, wgT_hbm, wuT_hbm, wd_hbm, c_ref, wmod_hbm,
            out_ref,
            x_ref, wqkv_ref, wo_ref, wguT_ref, wd_ref, wmod_ref,
            sems, xsems, z_ref, hb_ref,
            mod_ref, wqvT_ref, kwin_ref, qT_ref, vT_ref,
            sA, sB, mA, mB, oT_ref):
    step = pl.program_id(0)

    def cp(src, dst, i):
        return pltpu.make_async_copy(src, dst, sems.at[i])

    d_mod1 = cp(wmod_hbm.at[:, 0:2 * D], wmod_ref.at[:, 0:2 * D], 0)
    d_wk = cp(wqkv_hbm.at[:, D:2 * D], wqkv_ref.at[:, D:2 * D], 1)
    d_wq = cp(wqkv_hbm.at[:, 0:D], wqkv_ref.at[:, 0:D], 2)
    d_wv = cp(wqkv_hbm.at[:, 2 * D:3 * D], wqkv_ref.at[:, 2 * D:3 * D], 3)

    def d_x(b):
        r0 = pl.multiple_of(b * PB, PB)
        return pltpu.make_async_copy(x_hbm.at[pl.ds(r0, PB), :],
                                     x_ref.at[pl.ds(r0, PB), :], xsems.at[b])

    late = [
        cp(wmod_hbm.at[:, 2 * D:6 * D], wmod_ref.at[:, 2 * D:6 * D], 4),
        cp(wo_hbm, wo_ref, 5),
        cp(wgT_hbm.at[0:FA, :], wguT_ref.at[0:FA, :], 6),
        cp(wuT_hbm.at[0:FA, :], wguT_ref.at[FA:2 * FA, :], 7),
        cp(wgT_hbm.at[FA:F, :], wguT_ref.at[2 * FA:2 * FA + FT, :], 8),
        cp(wuT_hbm.at[FA:F, :], wguT_ref.at[2 * FA + FT:2 * F, :], 9),
        cp(wd_hbm, wd_ref, 10),
    ]

    def silu_c():
        c = jnp.broadcast_to(c_ref[...].astype(_F32), (8, D))
        return (c * jax.nn.sigmoid(c)).astype(_BF)

    nc = S // KC
    sub128 = jax.lax.broadcasted_iota(jnp.int32, (128, TQ), 0)

    def get_qm(u):
        h = u % H
        q0 = pl.multiple_of((u // H) * TQ, TQ)
        w = h // HPW
        st = jnp.minimum(w * (HPW * DH), D - 128)
        lo = h * DH - st
        q = qT_ref[pl.ds(pl.multiple_of(st, 8), 128), pl.ds(q0, TQ)]
        return w, jnp.where((sub128 >= lo) & (sub128 < lo + DH), q, 0.0).astype(_BF)

    def a_chunk(w, qm, c, s_ref, mx):
        sT = jnp.dot(kwin_ref[w, c * KC:(c + 1) * KC, :], qm,
                     preferred_element_type=_F32)
        s_ref[c * KC:(c + 1) * KC, :] = sT
        cm = jnp.max(sT.reshape(KC // 8, 8, TQ), axis=0)
        return cm if mx is None else jnp.maximum(mx, cm)

    @pl.when(step == 0)
    def _prep():
        d_mod1.start()
        d_wk.start()
        d_x(0).start()
        z_ref[0] = 0
        with _scope('w0'):
            d_mod1.wait()
        mod_ref[:, 0:2 * D] = jnp.dot(silu_c(), wmod_ref[:, 0:2 * D],
                                      preferred_element_type=_F32)
        with _scope('w1'):
            d_wk.wait()
            d_x(0).wait()
        d_wq.start()
        d_wv.start()
        d_x(1).start()

        def kpart(b):
            for t in range(PB // PRC):
                r0 = pl.multiple_of(b * PB + t * PRC, PRC)
                x = x_ref[pl.ds(r0, PRC), :].astype(_F32)
                h = _layernorm(x) * (1.0 + mod_ref[0:1, D:2 * D]) + mod_ref[0:1, 0:D]
                hb = h.astype(_BF)
                hb_ref[pl.ds(r0, PRC), :] = hb
                k = jnp.dot(hb, wqkv_ref[:, D:2 * D], preferred_element_type=_F32)
                for w in range(NW):
                    st = _win_start(w)
                    kwin_ref[w, pl.ds(r0, PRC), :] = k[:, st:st + 128].astype(_BF)

        row32 = jax.lax.broadcasted_iota(jnp.int32, (32, RC), 0)

        def qvpart(b):
            for t in range(PB // RC):
                r0 = pl.multiple_of(b * PB + t * RC, RC)
                hb = hb_ref[pl.ds(r0, RC), :]
                qv = jax.lax.dot_general(wqvT_ref[...], hb, _NT,
                                         preferred_element_type=_F32)
                qT_ref[:, pl.ds(r0, RC)] = qv[0:D] * QSCALE
                for hh in range(H):
                    lo = D + hh * DH
                    if lo + 32 <= 2 * D:
                        blk = qv[lo:lo + 32]
                    else:
                        blk = jnp.concatenate(
                            [qv[lo:lo + DH], jnp.zeros((32 - DH, RC), _F32)], axis=0)
                    blk = jnp.where(row32 < DH, blk, jnp.where(row32 == 31, 1.0, 0.0))
                    vT_ref[hh, :, pl.ds(r0, RC)] = blk.astype(_BF)

        with _scope('prep_k0'):
            kpart(0)

        with _scope('w2'):
            d_wq.wait()
            d_wv.wait()
        for b in range(2, S // PB):
            d_x(b).start()
        with _scope('prep_T'):
            wqvT_ref[0:D, :] = wqkv_ref[:, 0:D].astype(_F32).T.astype(_BF)
            wqvT_ref[D:2 * D, :] = wqkv_ref[:, 2 * D:3 * D].astype(_F32).T.astype(_BF)

        def body(b, carry):
            d_x(b + 1).wait()
            qvpart(b)
            kpart(b + 1)
            return carry

        with _scope('prep_loop'):
            jax.lax.fori_loop(0, S // PB - 1, body, 0)
        for d in late:
            d.start()
        qvpart(S // PB - 1)

        w0, qm0 = get_qm(jnp.int32(0))
        mx0 = None
        for c in range(nc):
            mx0 = a_chunk(w0, qm0, c, sA, mx0)
        mA[...] = jnp.max(mx0, axis=0, keepdims=True)

    z = pl.multiple_of(z_ref[0], 8)

    def b_chunk(h, c, s_ref, m, acc):
        p = jnp.exp2(s_ref[pl.ds(z + c * KC, KC), :] - m).astype(_BF)
        o = jnp.dot(vT_ref[h, :, c * KC:(c + 1) * KC], p,
                    preferred_element_type=_F32)
        return o if acc is None else acc + o

    def ab(u_a, s_w, m_w, h_b, s_r, m_r):
        w, qm = get_qm(u_a)
        m = m_r[...]
        mx = None
        acc = None
        for c in range(nc + SKEW):
            if c < nc:
                mx = a_chunk(w, qm, c, s_w, mx)
            if c >= SKEW:
                acc = b_chunk(h_b, c - SKEW, s_r, m, acc)
        m_w[...] = jnp.max(mx, axis=0, keepdims=True)
        return acc[0:DH] / acc[31:32]

    u0 = step * H

    def group(j, carry):
        for t in range(UPB // 2):
            h = j * UPB + 2 * t
            o0 = ab(u0 + h + 1, sB, mB, h, sA, mA)
            o1 = ab(jnp.minimum(u0 + h + 2, NQ * H - 1), sA, mA, h + 1, sB, mB)
            oT_ref[pl.ds(pl.multiple_of(h * DH, 8), 2 * DH), :] = (
                jnp.concatenate([o0, o1], axis=0))
        return carry

    with _scope('attn_loop'):
        jax.lax.fori_loop(0, H // UPB, group, 0)

    @pl.when(step == 0)
    def _late():
        for d in late:
            d.wait()
        mod_ref[:, 2 * D:6 * D] = jnp.dot(silu_c(), wmod_ref[:, 2 * D:6 * D],
                                          preferred_element_type=_F32)

    q0 = pl.multiple_of(step * TQ, TQ)
    nrc = FB // FRC
    nfb = TQ // FB

    def ffn_block(fb, carry):
        x1s = []
        for rc in range(nrc):
            c0 = pl.multiple_of(fb * FB + rc * FRC, FRC)
            o = oT_ref[:, pl.ds(c0, FRC)].T.astype(_BF)
            attn = jnp.dot(o, wo_ref[...], preferred_element_type=_F32)
            x = x_ref[pl.ds(pl.multiple_of(q0 + c0, FRC), FRC), :].astype(_F32)
            x1s.append(x + mod_ref[0:1, 2 * D:3 * D] * attn)
        acts = []
        for rc in range(nrc):
            h2 = (_layernorm(x1s[rc]) * (1.0 + mod_ref[0:1, 4 * D:5 * D])
                  + mod_ref[0:1, 3 * D:4 * D]).astype(_BF)
            gu = jax.lax.dot_general(h2, wguT_ref[...], _NT,
                                     preferred_element_type=_F32)
            a_main = jax.nn.gelu(gu[:, 0:FA], approximate=True) * gu[:, FA:2 * FA]
            a_tail = (jax.nn.gelu(gu[:, 2 * FA:2 * FA + FT], approximate=True)
                      * gu[:, 2 * FA + FT:2 * F])
            acts.append(jnp.concatenate([a_main, a_tail], axis=1).astype(_BF))
        for rc in range(nrc):
            c0 = pl.multiple_of(fb * FB + rc * FRC, FRC)
            y = jnp.dot(acts[rc], wd_ref[...], preferred_element_type=_F32)
            out_ref[pl.ds(c0, FRC), :] = (
                x1s[rc] + mod_ref[0:1, 5 * D:6 * D] * y).astype(out_ref.dtype)
        return carry

    with _scope('ffn'):
        jax.lax.fori_loop(0, nfb, ffn_block, 0)


@jax.jit
def pallas_adaLN_cond__mha_block__geglu_ffn__prompt_kernel(
    A_x: jax.Array,
    A_wqkv: jax.Array,
    A_wo: jax.Array,
    B_x: jax.Array,
    B_w_gate: jax.Array,
    B_w_up: jax.Array,
    B_w_down: jax.Array,
    c: jax.Array,
    w_mod: jax.Array,
):
    del B_x
    x = A_x.reshape(S, D)
    hbm = pl.BlockSpec(memory_space=pltpu.HBM)

    out = pl.pallas_call(
        _kernel,
        grid=(NQ,),
        in_specs=[hbm, hbm, hbm, hbm, hbm, hbm,
                  pl.BlockSpec((1, D), lambda i: (0, 0)), hbm],
        out_specs=pl.BlockSpec((TQ, D), lambda i: (i, 0)),
        out_shape=jax.ShapeDtypeStruct((S, D), A_x.dtype),
        scratch_shapes=[
            pltpu.VMEM((S, D), _BF),
            pltpu.VMEM((D, 3 * D), _BF),
            pltpu.VMEM((D, D), _BF),
            pltpu.VMEM((2 * F, D), _BF),
            pltpu.VMEM((F, D), _BF),
            pltpu.VMEM((D, 6 * D), _BF),
            pltpu.SemaphoreType.DMA((11,)),
            pltpu.SemaphoreType.DMA((S // PB,)),
            pltpu.SMEM((1,), jnp.int32),
            pltpu.VMEM((S, D), _BF),
            pltpu.VMEM((8, 6 * D), _F32),
            pltpu.VMEM((2 * D, D), _BF),
            pltpu.VMEM((NW, S, 128), _BF),
            pltpu.VMEM((D, S), _F32),
            pltpu.VMEM((H, 32, S), _BF),
            pltpu.VMEM((S, TQ), _F32),
            pltpu.VMEM((S, TQ), _F32),
            pltpu.VMEM((1, TQ), _F32),
            pltpu.VMEM((1, TQ), _F32),
            pltpu.VMEM((D, TQ), _F32),
        ],
        compiler_params=pltpu.CompilerParams(
            dimension_semantics=("arbitrary",),
            vmem_limit_bytes=110 * 1024 * 1024,
        ),
    )(x, A_wqkv, A_wo, B_w_gate.T, B_w_up.T, B_w_down, c, w_mod)
    return out.reshape(A_x.shape)
```

```python
import jax
import jax.numpy as jnp
import jax.experimental.pallas as pl
import jax.experimental.pallas.tpu as pltpu

S = 2048
D = 640
H = 32
DH = 20
F = 1728
FA = 1664
FT = F - FA
TQ = 256
NQ = S // TQ
KC = 128
NB = 4
SKEW = 3
UPB = 16
RC = 256
PB = 512
PRC = 128
FB = 256
FRC = 128
HPW = 6
NW = 6
EPS = 1e-5
LOG2E = 1.4426950408889634
QSCALE = (DH ** -0.5) * LOG2E

_NT = (((1,), (1,)), ((), ()))
_BF = jnp.bfloat16
_F32 = jnp.float32


class _scope:
    enabled = False

    def __init__(self, name):
        self._cm = jax.named_scope(name) if _scope.enabled else None

    def __enter__(self):
        if self._cm is not None:
            self._cm.__enter__()

    def __exit__(self, *a):
        if self._cm is not None:
            self._cm.__exit__(*a)


def _win_start(w):
    return min(w * HPW * DH, D - 128)


def _layernorm(x):
    m = jnp.mean(x, axis=-1, keepdims=True)
    xc = x - m
    v = jnp.mean(xc * xc, axis=-1, keepdims=True)
    return xc * jax.lax.rsqrt(v + EPS)


def _kernel(x_hbm, wqkv_hbm, wo_hbm, wgT_hbm, wuT_hbm, wd_hbm, c_ref, wmod_hbm,
            out_ref,
            x_ref, wqkv_ref, wo_ref, wguT_ref, wd_ref, wmod_ref,
            sems, xsems, z_ref, hb_ref,
            mod_ref, wqvT_ref, kwin_ref, qT_ref, vT_ref,
            sA, sB, s2, s3, mA, oT_ref):
    step = pl.program_id(0)

    def cp(src, dst, i):
        return pltpu.make_async_copy(src, dst, sems.at[i])

    d_mod1 = cp(wmod_hbm.at[:, 0:2 * D], wmod_ref.at[:, 0:2 * D], 0)
    d_wk = cp(wqkv_hbm.at[:, D:2 * D], wqkv_ref.at[:, D:2 * D], 1)
    d_wq = cp(wqkv_hbm.at[:, 0:D], wqkv_ref.at[:, 0:D], 2)
    d_wv = cp(wqkv_hbm.at[:, 2 * D:3 * D], wqkv_ref.at[:, 2 * D:3 * D], 3)

    def d_x(b):
        r0 = pl.multiple_of(b * PB, PB)
        return pltpu.make_async_copy(x_hbm.at[pl.ds(r0, PB), :],
                                     x_ref.at[pl.ds(r0, PB), :], xsems.at[b])

    late = [
        cp(wmod_hbm.at[:, 2 * D:6 * D], wmod_ref.at[:, 2 * D:6 * D], 4),
        cp(wo_hbm, wo_ref, 5),
        cp(wgT_hbm.at[0:FA, :], wguT_ref.at[0:FA, :], 6),
        cp(wuT_hbm.at[0:FA, :], wguT_ref.at[FA:2 * FA, :], 7),
        cp(wgT_hbm.at[FA:F, :], wguT_ref.at[2 * FA:2 * FA + FT, :], 8),
        cp(wuT_hbm.at[FA:F, :], wguT_ref.at[2 * FA + FT:2 * F, :], 9),
        cp(wd_hbm, wd_ref, 10),
    ]

    def silu_c():
        c = jnp.broadcast_to(c_ref[...].astype(_F32), (8, D))
        return (c * jax.nn.sigmoid(c)).astype(_BF)

    nc = S // KC
    sub128 = jax.lax.broadcasted_iota(jnp.int32, (128, TQ), 0)

    def get_qm(u):
        h = u % H
        q0 = pl.multiple_of((u // H) * TQ, TQ)
        w = h // HPW
        st = jnp.minimum(w * (HPW * DH), D - 128)
        lo = h * DH - st
        q = qT_ref[pl.ds(pl.multiple_of(st, 8), 128), pl.ds(q0, TQ)]
        return w, jnp.where((sub128 >= lo) & (sub128 < lo + DH), q, 0.0).astype(_BF)

    def a_chunk(w, qm, c, s_ref, mx):
        sT = jnp.dot(kwin_ref[w, c * KC:(c + 1) * KC, :], qm,
                     preferred_element_type=_F32)
        s_ref[c * KC:(c + 1) * KC, :] = sT
        cm = jnp.max(sT.reshape(KC // 8, 8, TQ), axis=0)
        return cm if mx is None else jnp.maximum(mx, cm)

    @pl.when(step == 0)
    def _prep():
        d_mod1.start()
        d_wk.start()
        d_x(0).start()
        z_ref[0] = 0
        with _scope('w0'):
            d_mod1.wait()
        mod_ref[:, 0:2 * D] = jnp.dot(silu_c(), wmod_ref[:, 0:2 * D],
                                      preferred_element_type=_F32)
        with _scope('w1'):
            d_wk.wait()
            d_x(0).wait()
        d_wq.start()
        d_wv.start()
        d_x(1).start()

        def kpart(b):
            for t in range(PB // PRC):
                r0 = pl.multiple_of(b * PB + t * PRC, PRC)
                x = x_ref[pl.ds(r0, PRC), :].astype(_F32)
                h = _layernorm(x) * (1.0 + mod_ref[0:1, D:2 * D]) + mod_ref[0:1, 0:D]
                hb = h.astype(_BF)
                hb_ref[pl.ds(r0, PRC), :] = hb
                k = jnp.dot(hb, wqkv_ref[:, D:2 * D], preferred_element_type=_F32)
                for w in range(NW):
                    st = _win_start(w)
                    kwin_ref[w, pl.ds(r0, PRC), :] = k[:, st:st + 128].astype(_BF)

        row32 = jax.lax.broadcasted_iota(jnp.int32, (32, RC), 0)

        def qvpart(b):
            for t in range(PB // RC):
                r0 = pl.multiple_of(b * PB + t * RC, RC)
                hb = hb_ref[pl.ds(r0, RC), :]
                qv = jax.lax.dot_general(wqvT_ref[...], hb, _NT,
                                         preferred_element_type=_F32)
                qT_ref[:, pl.ds(r0, RC)] = qv[0:D] * QSCALE
                for hh in range(H):
                    lo = D + hh * DH
                    if lo + 32 <= 2 * D:
                        blk = qv[lo:lo + 32]
                    else:
                        blk = jnp.concatenate(
                            [qv[lo:lo + DH], jnp.zeros((32 - DH, RC), _F32)], axis=0)
                    blk = jnp.where(row32 < DH, blk, jnp.where(row32 == 31, 1.0, 0.0))
                    vT_ref[hh, :, pl.ds(r0, RC)] = blk.astype(_BF)

        with _scope('prep_k0'):
            kpart(0)

        with _scope('w2'):
            d_wq.wait()
            d_wv.wait()
        for b in range(2, S // PB):
            d_x(b).start()
        with _scope('prep_T'):
            wqvT_ref[0:D, :] = wqkv_ref[:, 0:D].astype(_F32).T.astype(_BF)
            wqvT_ref[D:2 * D, :] = wqkv_ref[:, 2 * D:3 * D].astype(_F32).T.astype(_BF)

        def body(b, carry):
            d_x(b + 1).wait()
            qvpart(b)
            kpart(b + 1)
            return carry

        with _scope('prep_loop'):
            jax.lax.fori_loop(0, S // PB - 1, body, 0)
        for d in late:
            d.start()
        qvpart(S // PB - 1)

        w0, qm0 = get_qm(jnp.int32(0))
        mx0 = None
        for c in range(nc):
            mx0 = a_chunk(w0, qm0, c, sA, mx0)
        mA[...] = jnp.max(mx0, axis=0, keepdims=True)

    z = pl.multiple_of(z_ref[0], 8)

    def b_chunk(h, c, s_ref, m, acc):
        p = jnp.exp2(s_ref[pl.ds(z + c * KC, KC), :] - m).astype(_BF)
        o = jnp.dot(vT_ref[h, :, c * KC:(c + 1) * KC], p,
                    preferred_element_type=_F32)
        return o if acc is None else acc + o

    u0 = step * H
    sbufs = (sA, sB, s2, s3)

    def group(j, carry):
        hb = j * UPB
        ms = {0: mA[...]}
        qms = {}
        mxs = {}
        accs = {}
        outs = {}
        for t in range(UPB * nc + SKEW):
            if t < UPB * nc:
                k, c = t // nc + 1, t % nc
                if c == 0:
                    qms[k] = get_qm(jnp.minimum(u0 + hb + k, NQ * H - 1))
                    mxs[k] = None
                w, qm = qms[k]
                mxs[k] = a_chunk(w, qm, c, sbufs[k % NB], mxs[k])
                if c == nc - 1:
                    ms[k] = jnp.max(mxs[k], axis=0, keepdims=True)
                    if k == UPB:
                        mA[...] = ms[k]
            if t >= SKEW:
                k, c = (t - SKEW) // nc, (t - SKEW) % nc
                if c == 0:
                    accs[k] = None
                accs[k] = b_chunk(hb + k, c, sbufs[k % NB], ms[k], accs[k])
                if c == nc - 1:
                    outs[k] = accs[k][0:DH] / accs[k][31:32]
                    if k % 2 == 1:
                        oT_ref[pl.ds(pl.multiple_of((hb + k - 1) * DH, 8), 2 * DH), :] = (
                            jnp.concatenate([outs[k - 1], outs[k]], axis=0))
        return carry

    with _scope('attn_loop'):
        jax.lax.fori_loop(0, H // UPB, group, 0)

    @pl.when(step == 0)
    def _late():
        for d in late:
            d.wait()
        mod_ref[:, 2 * D:6 * D] = jnp.dot(silu_c(), wmod_ref[:, 2 * D:6 * D],
                                          preferred_element_type=_F32)

    q0 = pl.multiple_of(step * TQ, TQ)
    nrc = FB // FRC
    nfb = TQ // FB

    def ffn_block(fb, carry):
        x1s = []
        for rc in range(nrc):
            c0 = pl.multiple_of(fb * FB + rc * FRC, FRC)
            o = oT_ref[:, pl.ds(c0, FRC)].T.astype(_BF)
            attn = jnp.dot(o, wo_ref[...], preferred_element_type=_F32)
            x = x_ref[pl.ds(pl.multiple_of(q0 + c0, FRC), FRC), :].astype(_F32)
            x1s.append(x + mod_ref[0:1, 2 * D:3 * D] * attn)
        acts = []
        for rc in range(nrc):
            h2 = (_layernorm(x1s[rc]) * (1.0 + mod_ref[0:1, 4 * D:5 * D])
                  + mod_ref[0:1, 3 * D:4 * D]).astype(_BF)
            gu = jax.lax.dot_general(h2, wguT_ref[...], _NT,
                                     preferred_element_type=_F32)
            a_main = jax.nn.gelu(gu[:, 0:FA], approximate=True) * gu[:, FA:2 * FA]
            a_tail = (jax.nn.gelu(gu[:, 2 * FA:2 * FA + FT], approximate=True)
                      * gu[:, 2 * FA + FT:2 * F])
            acts.append(jnp.concatenate([a_main, a_tail], axis=1).astype(_BF))
        for rc in range(nrc):
            c0 = pl.multiple_of(fb * FB + rc * FRC, FRC)
            y = jnp.dot(acts[rc], wd_ref[...], preferred_element_type=_F32)
            out_ref[pl.ds(c0, FRC), :] = (
                x1s[rc] + mod_ref[0:1, 5 * D:6 * D] * y).astype(out_ref.dtype)
        return carry

    with _scope('ffn'):
        jax.lax.fori_loop(0, nfb, ffn_block, 0)


@jax.jit
def pallas_adaLN_cond__mha_block__geglu_ffn__prompt_kernel(
    A_x: jax.Array,
    A_wqkv: jax.Array,
    A_wo: jax.Array,
    B_x: jax.Array,
    B_w_gate: jax.Array,
    B_w_up: jax.Array,
    B_w_down: jax.Array,
    c: jax.Array,
    w_mod: jax.Array,
):
    del B_x
    x = A_x.reshape(S, D)
    hbm = pl.BlockSpec(memory_space=pltpu.HBM)

    out = pl.pallas_call(
        _kernel,
        grid=(NQ,),
        in_specs=[hbm, hbm, hbm, hbm, hbm, hbm,
                  pl.BlockSpec((1, D), lambda i: (0, 0)), hbm],
        out_specs=pl.BlockSpec((TQ, D), lambda i: (i, 0)),
        out_shape=jax.ShapeDtypeStruct((S, D), A_x.dtype),
        scratch_shapes=[
            pltpu.VMEM((S, D), _BF),
            pltpu.VMEM((D, 3 * D), _BF),
            pltpu.VMEM((D, D), _BF),
            pltpu.VMEM((2 * F, D), _BF),
            pltpu.VMEM((F, D), _BF),
            pltpu.VMEM((D, 6 * D), _BF),
            pltpu.SemaphoreType.DMA((11,)),
            pltpu.SemaphoreType.DMA((S // PB,)),
            pltpu.SMEM((1,), jnp.int32),
            pltpu.VMEM((S, D), _BF),
            pltpu.VMEM((8, 6 * D), _F32),
            pltpu.VMEM((2 * D, D), _BF),
            pltpu.VMEM((NW, S, 128), _BF),
            pltpu.VMEM((D, S), _F32),
            pltpu.VMEM((H, 32, S), _BF),
            pltpu.VMEM((S, TQ), _F32),
            pltpu.VMEM((S, TQ), _F32),
            pltpu.VMEM((S, TQ), _F32),
            pltpu.VMEM((S, TQ), _F32),
            pltpu.VMEM((1, TQ), _F32),
            pltpu.VMEM((D, TQ), _F32),
        ],
        compiler_params=pltpu.CompilerParams(
            dimension_semantics=("arbitrary",),
            vmem_limit_bytes=110 * 1024 * 1024,
        ),
    )(x, A_wqkv, A_wo, B_w_gate.T, B_w_up.T, B_w_down, c, w_mod)
    return out.reshape(A_x.shape)
```

```python
import jax
import jax.numpy as jnp
import jax.experimental.pallas as pl
import jax.experimental.pallas.tpu as pltpu

S = 2048
D = 640
H = 32
DH = 20
F = 1728
FA = 1664
FT = F - FA
TQ = 256
NQ = S // TQ
KC = 128
NB = 4
SKEW = 3
UPB = 16
RC = 512
PB = 512
PRC = 256
FRC = 128
HPW = 6
NW = 6
EPS = 1e-5
LOG2E = 1.4426950408889634
QSCALE = (DH ** -0.5) * LOG2E

_NT = (((1,), (1,)), ((), ()))
_BF = jnp.bfloat16
_F32 = jnp.float32


def _win_start(w):
    return min(w * HPW * DH, D - 128)


def _layernorm(x):
    m = jnp.mean(x, axis=-1, keepdims=True)
    xc = x - m
    v = jnp.mean(xc * xc, axis=-1, keepdims=True)
    return xc * jax.lax.rsqrt(v + EPS)


def _kernel(x_hbm, wqkv_hbm, wo_hbm, wgT_hbm, wuT_hbm, wd_hbm, c_ref, wmod_hbm,
            out_ref,
            x_ref, wq_ref, wk_ref, wv_ref, wo_ref, wguT_ref, wd_ref,
            wmod1_ref, wmod2_ref,
            sems, xsems, z_ref, hb_ref,
            mod_ref, wqvT_ref, kwin_ref, qT_ref, vT_ref,
            s0, s1, s2, s3, mcar, oT_ref):
    step = pl.program_id(0)

    def cp(src, dst, i):
        return pltpu.make_async_copy(src, dst, sems.at[i])

    d_mod1 = cp(wmod_hbm.at[:, 0:2 * D], wmod1_ref, 0)
    d_wk = cp(wqkv_hbm.at[:, D:2 * D], wk_ref, 1)
    d_wq = cp(wqkv_hbm.at[:, 0:D], wq_ref, 2)
    d_wv = cp(wqkv_hbm.at[:, 2 * D:3 * D], wv_ref, 3)
    d_mod2 = cp(wmod_hbm.at[:, 2 * D:6 * D], wmod2_ref, 4)
    late = [
        cp(wo_hbm, wo_ref, 5),
        cp(wgT_hbm.at[0:FA, :], wguT_ref.at[0:FA, :], 6),
        cp(wuT_hbm.at[0:FA, :], wguT_ref.at[FA:2 * FA, :], 7),
        cp(wgT_hbm.at[FA:F, :], wguT_ref.at[2 * FA:2 * FA + FT, :], 8),
        cp(wuT_hbm.at[FA:F, :], wguT_ref.at[2 * FA + FT:2 * F, :], 9),
        cp(wd_hbm, wd_ref, 10),
    ]

    def d_x(b):
        r0 = pl.multiple_of(b * PB, PB)
        return pltpu.make_async_copy(x_hbm.at[pl.ds(r0, PB), :],
                                     x_ref.at[pl.ds(r0, PB), :], xsems.at[b])

    def silu_c():
        c = jnp.broadcast_to(c_ref[...].astype(_F32), (8, D))
        return (c * jax.nn.sigmoid(c)).astype(_BF)

    nc = S // KC
    sub128 = jax.lax.broadcasted_iota(jnp.int32, (128, TQ), 0)

    def get_qm(u):
        h = u % H
        q0 = pl.multiple_of((u // H) * TQ, TQ)
        w = h // HPW
        st = jnp.minimum(w * (HPW * DH), D - 128)
        lo = h * DH - st
        q = qT_ref[pl.ds(pl.multiple_of(st, 8), 128), pl.ds(q0, TQ)]
        return w, jnp.where((sub128 >= lo) & (sub128 < lo + DH), q, 0.0).astype(_BF)

    def a_chunk(w, qm, c, s_ref, mx):
        sT = jnp.dot(kwin_ref[w, c * KC:(c + 1) * KC, :], qm,
                     preferred_element_type=_F32)
        s_ref[c * KC:(c + 1) * KC, :] = sT
        cm = jnp.max(sT.reshape(KC // 8, 8, TQ), axis=0)
        return cm if mx is None else jnp.maximum(mx, cm)

    @pl.when(step == 0)
    def _prep():
        d_mod1.start()
        d_wk.start()
        d_x(0).start()
        d_wq.start()
        d_wv.start()
        d_x(1).start()
        z_ref[0] = 0
        d_mod1.wait()
        mod_ref[:, 0:2 * D] = jnp.dot(silu_c(), wmod1_ref[...],
                                      preferred_element_type=_F32)
        d_wk.wait()
        d_x(0).wait()

        def kpart(b):
            for t in range(PB // PRC):
                r0 = pl.multiple_of(b * PB + t * PRC, PRC)
                x = x_ref[pl.ds(r0, PRC), :].astype(_F32)
                h = _layernorm(x) * (1.0 + mod_ref[0:1, D:2 * D]) + mod_ref[0:1, 0:D]
                hb = h.astype(_BF)
                hb_ref[pl.ds(r0, PRC), :] = hb
                k = jnp.dot(hb, wk_ref[...], preferred_element_type=_F32)
                for w in range(NW):
                    st = _win_start(w)
                    kwin_ref[w, pl.ds(r0, PRC), :] = k[:, st:st + 128].astype(_BF)

        row32 = jax.lax.broadcasted_iota(jnp.int32, (32, RC), 0)

        def qvpart(b):
            for t in range(PB // RC):
                r0 = pl.multiple_of(b * PB + t * RC, RC)
                hb = hb_ref[pl.ds(r0, RC), :]
                qv = jax.lax.dot_general(wqvT_ref[...], hb, _NT,
                                         preferred_element_type=_F32)
                qT_ref[:, pl.ds(r0, RC)] = qv[0:D] * QSCALE
                for hh in range(H):
                    lo = D + hh * DH
                    if lo + 32 <= 2 * D:
                        blk = qv[lo:lo + 32]
                    else:
                        blk = jnp.concatenate(
                            [qv[lo:lo + DH], jnp.zeros((32 - DH, RC), _F32)], axis=0)
                    blk = jnp.where(row32 < DH, blk, jnp.where(row32 == 31, 1.0, 0.0))
                    vT_ref[hh, :, pl.ds(r0, RC)] = blk.astype(_BF)

        kpart(0)

        d_wq.wait()
        d_wv.wait()
        for b in range(2, S // PB):
            d_x(b).start()
        d_mod2.start()
        wqvT_ref[0:D, :] = wq_ref[...].astype(_F32).T.astype(_BF)
        wqvT_ref[D:2 * D, :] = wv_ref[...].astype(_F32).T.astype(_BF)

        def body(b, carry):
            d_x(b + 1).wait()
            qvpart(b)
            kpart(b + 1)
            return carry

        jax.lax.fori_loop(0, S // PB - 1, body, 0)
        for d in late:
            d.start()
        d_mod2.wait()
        qvpart(S // PB - 1)
        mod_ref[:, 2 * D:6 * D] = jnp.dot(silu_c(), wmod2_ref[...],
                                          preferred_element_type=_F32)

        w0, qm0 = get_qm(jnp.int32(0))
        mx0 = None
        for c in range(nc):
            mx0 = a_chunk(w0, qm0, c, s0, mx0)
        mcar[...] = jnp.max(mx0, axis=0, keepdims=True)

    z = pl.multiple_of(z_ref[0], 8)

    def b_chunk(h, c, s_ref, m, acc):
        p = jnp.exp2(s_ref[pl.ds(z + c * KC, KC), :] - m).astype(_BF)
        o = jnp.dot(vT_ref[h, :, c * KC:(c + 1) * KC], p,
                    preferred_element_type=_F32)
        return o if acc is None else acc + o

    u0 = step * H
    sbufs = (s0, s1, s2, s3)

    def group(j, carry):
        hb = j * UPB
        ms = {0: mcar[...]}
        qms, mxs, accs, outs = {}, {}, {}, {}
        for t in range(UPB * nc + SKEW):
            if t < UPB * nc:
                k, c = t // nc + 1, t % nc
                if c == 0:
                    qms[k] = get_qm(jnp.minimum(u0 + hb + k, NQ * H - 1))
                    mxs[k] = None
                w, qm = qms[k]
                mxs[k] = a_chunk(w, qm, c, sbufs[k % NB], mxs[k])
                if c == nc - 1:
                    ms[k] = jnp.max(mxs[k], axis=0, keepdims=True)
                    if k == UPB:
                        mcar[...] = ms[k]
            if t >= SKEW:
                k, c = (t - SKEW) // nc, (t - SKEW) % nc
                if c == 0:
                    accs[k] = None
                accs[k] = b_chunk(hb + k, c, sbufs[k % NB], ms[k], accs[k])
                if c == nc - 1:
                    outs[k] = accs[k][0:DH] / accs[k][31:32]
                    if k % 2 == 1:
                        oT_ref[pl.ds(pl.multiple_of((hb + k - 1) * DH, 8), 2 * DH), :] = (
                            jnp.concatenate([outs[k - 1], outs[k]], axis=0))
        return carry

    jax.lax.fori_loop(0, H // UPB, group, 0)

    @pl.when(step == 0)
    def _late():
        for d in late:
            d.wait()

    q0 = pl.multiple_of(step * TQ, TQ)
    nrc = TQ // FRC
    x1s = []
    for rc in range(nrc):
        o = oT_ref[:, rc * FRC:(rc + 1) * FRC].T.astype(_BF)
        attn = jnp.dot(o, wo_ref[...], preferred_element_type=_F32)
        x = x_ref[pl.ds(pl.multiple_of(q0 + rc * FRC, FRC), FRC), :].astype(_F32)
        x1s.append(x + mod_ref[0:1, 2 * D:3 * D] * attn)
    acts = []
    for rc in range(nrc):
        h2 = (_layernorm(x1s[rc]) * (1.0 + mod_ref[0:1, 4 * D:5 * D])
              + mod_ref[0:1, 3 * D:4 * D]).astype(_BF)
        gu = jax.lax.dot_general(h2, wguT_ref[...], _NT,
                                 preferred_element_type=_F32)
        a_main = jax.nn.gelu(gu[:, 0:FA], approximate=True) * gu[:, FA:2 * FA]
        a_tail = (jax.nn.gelu(gu[:, 2 * FA:2 * FA + FT], approximate=True)
                  * gu[:, 2 * FA + FT:2 * F])
        acts.append(jnp.concatenate([a_main, a_tail], axis=1).astype(_BF))
    for rc in range(nrc):
        y = jnp.dot(acts[rc], wd_ref[...], preferred_element_type=_F32)
        out_ref[rc * FRC:(rc + 1) * FRC, :] = (
            x1s[rc] + mod_ref[0:1, 5 * D:6 * D] * y).astype(out_ref.dtype)


@jax.jit
def pallas_adaLN_cond__mha_block__geglu_ffn__prompt_kernel(
    A_x: jax.Array,
    A_wqkv: jax.Array,
    A_wo: jax.Array,
    B_x: jax.Array,
    B_w_gate: jax.Array,
    B_w_up: jax.Array,
    B_w_down: jax.Array,
    c: jax.Array,
    w_mod: jax.Array,
):
    del B_x
    x = A_x.reshape(S, D)
    hbm = pl.BlockSpec(memory_space=pltpu.HBM)

    out = pl.pallas_call(
        _kernel,
        grid=(NQ,),
        in_specs=[hbm, hbm, hbm, hbm, hbm, hbm,
                  pl.BlockSpec((1, D), lambda i: (0, 0)), hbm],
        out_specs=pl.BlockSpec((TQ, D), lambda i: (i, 0)),
        out_shape=jax.ShapeDtypeStruct((S, D), A_x.dtype),
        scratch_shapes=[
            pltpu.VMEM((S, D), _BF),
            pltpu.VMEM((D, D), _BF),
            pltpu.VMEM((D, D), _BF),
            pltpu.VMEM((D, D), _BF),
            pltpu.VMEM((D, D), _BF),
            pltpu.VMEM((2 * F, D), _BF),
            pltpu.VMEM((F, D), _BF),
            pltpu.VMEM((D, 2 * D), _BF),
            pltpu.VMEM((D, 4 * D), _BF),
            pltpu.SemaphoreType.DMA((11,)),
            pltpu.SemaphoreType.DMA((S // PB,)),
            pltpu.SMEM((1,), jnp.int32),
            pltpu.VMEM((S, D), _BF),
            pltpu.VMEM((8, 6 * D), _F32),
            pltpu.VMEM((2 * D, D), _BF),
            pltpu.VMEM((NW, S, 128), _BF),
            pltpu.VMEM((D, S), _F32),
            pltpu.VMEM((H, 32, S), _BF),
            pltpu.VMEM((S, TQ), _F32),
            pltpu.VMEM((S, TQ), _F32),
            pltpu.VMEM((S, TQ), _F32),
            pltpu.VMEM((S, TQ), _F32),
            pltpu.VMEM((1, TQ), _F32),
            pltpu.VMEM((D, TQ), _F32),
        ],
        compiler_params=pltpu.CompilerParams(
            dimension_semantics=("arbitrary",),
            vmem_limit_bytes=110 * 1024 * 1024,
        ),
    )(x, A_wqkv, A_wo, B_w_gate.T, B_w_up.T, B_w_down, c, w_mod)
    return out.reshape(A_x.shape)
```
